```python
import os as _os
_os.environ.setdefault("JAX_PLATFORMS", "cpu")
import jax
import jax.numpy as jnp

def _softmax(x, axis=-1):
    return jax.nn.softmax(x, axis=axis)
def _gelu(x):
    return jax.nn.gelu(x, approximate=True)
def _silu(x):
    return jax.nn.silu(x)
def _sigmoid(x):
    return jax.nn.sigmoid(x)
def _layernorm(x, axis=-1, eps=1e-5):
    m = jnp.mean(x, axis=axis, keepdims=True)
    v = jnp.var(x, axis=axis, keepdims=True)
    return (x - m) / jnp.sqrt(v + eps)
def _scatter_add(tgt, idx, src, axis=0):
    return tgt.at[idx].add(src)
def _segment_sum(src, seg, n):
    return jax.ops.segment_sum(src, seg, n)
class _Rng:
    def __init__(self, key):
        self._k = key
    def _next(self):
        self._k, sub = jax.random.split(self._k)
        return sub
    def normal(self, shape):
        return jax.random.normal(self._next(), shape, dtype=jnp.bfloat16)
    def randint(self, lo, hi, shape):
        return jax.random.randint(self._next(), shape, lo, hi, dtype=jnp.int32)
    def uniform(self, shape, lo=0.0, hi=1.0):
        return jax.random.uniform(self._next(), shape, jnp.bfloat16, lo, hi)
    def permutation(self, n):
        return jax.random.permutation(self._next(), n)


kernel_name = 'concat_heads__mha_block_cached__gqa_block_cached__decode'

def setup_inputs():
    _rng = _Rng(jax.random.key(int.from_bytes(__import__("os").urandom(4), "little")))
    _w = (lambda a: (lambda t: t.astype(jnp.bfloat16) if jnp.issubdtype(t.dtype, jnp.floating) else t)(jnp.asarray(a)))
    def _A_setup():
        B, Sq, D = 1, 1, 512
        H, Sk, Dh = 32, 4096, 128
        return {
            "x": _w((lambda *s: _rng.normal(s) * 0.8)(B, Sq, D)),
            "k_cache": _w((lambda *s: _rng.normal(s) * 0.8)(B, H, Sk, Dh)),
            "v_cache": _w((lambda *s: _rng.normal(s) * 0.05)(B, H, Sk, Dh)),
            "wq": _w((lambda *s: _rng.normal(s) * 0.8)(D, H * Dh) * (D ** -0.5)),
            "wo": _w((lambda *s: _rng.normal(s) * 0.05)(H * Dh, D) * ((H * Dh) ** -0.5)),
        }
    _A_in = _A_setup()

    def _B_setup():
        B, Sq, D = 1, 1, 512
        Hq, Hkv, Sk, Dh = 32, 32, 4096, 128
        assert Hq % Hkv == 0, (Hq, Hkv)
        return {
            "x": _w((lambda *s: _rng.normal(s) * 0.8)(B, Sq, D)),
            "k_cache": _w((lambda *s: _rng.normal(s) * 0.8)(B, Hkv, Sk, Dh)),
            "v_cache": _w((lambda *s: _rng.normal(s) * 0.05)(B, Hkv, Sk, Dh)),
            "wq": _w((lambda *s: _rng.normal(s) * 0.8)(D, Hq * Dh) * (D ** -0.5)),
            "wo": _w((lambda *s: _rng.normal(s) * 0.05)(Hq * Dh, D) * ((Hq * Dh) ** -0.5)),
        }
    _B_in = _B_setup()

    return {
        "A_x": _A_in["x"],
        "A_k_cache": _A_in["k_cache"],
        "A_v_cache": _A_in["v_cache"],
        "A_wq": _A_in["wq"],
        "A_wo": _A_in["wo"],
        "B_x": _B_in["x"],
        "B_k_cache": _B_in["k_cache"],
        "B_v_cache": _B_in["v_cache"],
        "B_wq": _B_in["wq"],
        "B_wo": _B_in["wo"],
    }

def reference(A_x, A_k_cache, A_v_cache, A_wq, A_wo, B_x, B_k_cache, B_v_cache, B_wq, B_wo):
    def _A_ref(x, k_cache, v_cache, wq, wo):
        B, Sq, D = x.shape
        H, Dh = 32, 128
        q = (lambda x, *d: x.transpose(*d))((x @ wq).reshape(B, Sq, H, Dh), 0, 2, 1, 3)
        scores = jnp.einsum("bhqd,bhkd->bhqk", q, k_cache) * (Dh ** -0.5)
        p = _softmax(scores, axis=-1)
        o = jnp.einsum("bhqk,bhkd->bhqd", p, v_cache)
        return (lambda x, *d: x.transpose(*d))(o, 0, 2, 1, 3).reshape(B, Sq, H * Dh) @ wo

    def _B_ref(x, k_cache, v_cache, wq, wo):
        B, Sq, D = x.shape
        Hq, Dh = 32, 128
        Hkv = k_cache.shape[1]
        rep = Hq // Hkv
        q = (lambda x, *d: x.transpose(*d))((x @ wq).reshape(B, Sq, Hq, Dh), 0, 2, 1, 3)
        k = jnp.repeat(k_cache, rep, axis=1)
        v = jnp.repeat(v_cache, rep, axis=1)
        scores = jnp.einsum("bhqd,bhkd->bhqk", q, k) * (Dh ** -0.5)
        p = _softmax(scores, axis=-1)
        o = jnp.einsum("bhqk,bhkd->bhqd", p, v)
        return (lambda x, *d: x.transpose(*d))(o, 0, 2, 1, 3).reshape(B, Sq, Hq * Dh) @ wo

    a = _A_ref(A_x, A_k_cache, A_v_cache, A_wq, A_wo)
    b = _B_ref(B_x, B_k_cache, B_v_cache, B_wq, B_wo)
    return jnp.concatenate([a, b], axis=-1)
```

```python
import functools
import jax, jax.numpy as jnp
from jax import lax
import jax.experimental.pallas as pl
import jax.experimental.pallas.tpu as pltpu

H, SK, DH, D = 32, 4096, 128, 512
U = 128
NS = 8
F32, BF16 = jnp.float32, jnp.bfloat16


def make(order=(0, 4, 2, 6, 1, 5, 3, 7), prio=(0, 1, 0, 1, 0, 1, 0, 1), hs=2, L0=2, L1=4, R=8,
         gmajor=False, compute=True, flags=None, issue_first=True, **cp):
    steps = [list(range(s, s + hs)) for s in range(0, NS, hs)]
    scale = DH ** -0.5

    def kern(ax, ak, av, awq, awo, bx, bk, bv, bwq, bwo, o_ref,
             xbuf, wqbuf, kvbuf, wobuf, q_s, s_s, m_s, l_s, o_s, sems, xsem):
        row = lax.broadcasted_iota(jnp.int32, (8, DH), 0)
        lane = lax.broadcasted_iota(jnp.int32, (8, DH), 1)

        def split(i):
            return (i // 32, i % 32) if gmajor else (i % 4, i // 4)

        def wq_copy(t, w):
            def f(i, j):
                seg = order[j]
                idx = (pl.ds(pl.multiple_of(64 * seg + 8 * (i // 2), 8), 8),
                       pl.ds(pl.multiple_of((i % 2) * 2048, 2048), 2048))
                return pltpu.make_async_copy(w.at[idx], wqbuf.at[(t,) + idx], sems.at[i % R, j])
            return f

        def kv_copy(r):
            def f(i, j):
                seg = order[j]
                g, rb = split(i)
                return pltpu.make_async_copy(
                    r.at[0, 4 * seg + g, pl.ds(pl.multiple_of(rb * U, U), U)],
                    kvbuf.at[i % R, j], sems.at[i % R, j])
            return f

        def wo_copy(w):
            def f(i, j):
                seg = order[j]
                return pltpu.make_async_copy(
                    w.at[pl.ds(pl.multiple_of(512 * seg + 32 * i, 32), 32)],
                    wobuf.at[i % R, pl.ds(32 * j, 32)], sems.at[i % R, j])
            return f

        def q_part(t, i):
            x8 = jnp.broadcast_to(xbuf[t, 0], (8, D))
            r = jnp.dot(x8, wqbuf[t, :, pl.ds(pl.multiple_of(256 * i, 256), 256)], preferred_element_type=F32)
            for e in range(2):
                g = 2 * (i % 2) + e
                q_s[t, pl.ds(8 * g + i // 2, 1), :] = r[0:1, e * DH:(e + 1) * DH]

        def no_compute(i, carry):
            for _ in steps:
                yield
            return carry

        def q_compute(t):
            def f(i, carry):
                yield
                q_part(t, i)
                for _ in steps[1:]:
                    yield
                return carry
            return f

        def k_compute(t):
            def f(i, carry):
                g, _ = split(i)
                q = q_s[t, pl.ds(pl.multiple_of(8 * g, 8), 8), :].astype(BF16)
                s = None
                for st in steps:
                    yield
                    for j in st:
                        r = lax.dot_general(q, kvbuf[i % R, j], (((1,), (1,)), ((), ())), preferred_element_type=F32)
                        s = r if s is None else jnp.where(row == order[j], r, s)
                s = s * scale
                s_s[i] = s
                m_s[g] = jnp.maximum(m_s[g], s)
                return carry
            return f

        def v_compute(i, carry):
            g, _ = split(i)
            p = jnp.exp(s_s[i] - m_s[g])
            l_s[g] += p
            pb = p.astype(BF16)
            o = None
            for st in steps:
                yield
                for j in st:
                    r = jnp.dot(pb, kvbuf[i % R, j], preferred_element_type=F32)
                    o = r if o is None else jnp.where(row == order[j], r, o)
            o_s[g] += o
            return carry

        def wo_compute(extra=None):
            def f(i, acc):
                g, c = i // 4, i % 4
                og = o_s[g]
                lhs = []
                for half in range(2):
                    d = None
                    for jj in range(4):
                        seg = order[4 * half + jj]
                        piece = pltpu.roll(jnp.broadcast_to(og[seg:seg + 1, :], (8, DH)), (32 * (jj - c)) % DH, 1)
                        d = piece if d is None else jnp.where(lane // 32 == jj, piece, d)
                    lhs.append(d.astype(BF16))
                for st in steps:
                    yield
                    if extra is not None and st is steps[0]:
                        extra(i)
                    for half in range(2):
                        if 4 * half + 3 in st:
                            acc = acc + jnp.dot(lhs[half], wobuf[i % R, pl.ds(128 * half, 128), :], preferred_element_type=F32)
                return acc
            return f

        def k_begin():
            m_s[...] = jnp.full(m_s.shape, -jnp.inf, F32)

        def v_begin():
            for g in range(4):
                m_s[g] = jnp.broadcast_to(jnp.max(m_s[g], axis=-1, keepdims=True), (8, DH))
            l_s[...] = jnp.zeros(l_s.shape, F32)
            o_s[...] = jnp.zeros(o_s.shape, F32)

        def wo_begin():
            for g in range(4):
                o_s[g] = o_s[g] / jnp.sum(l_s[g], axis=-1, keepdims=True)
            return jnp.zeros((8, D), F32)

        def wo_end(t):
            def f(acc):
                o_ref[0, :, pl.ds(t * D, D)] = acc[0:1, :].astype(o_ref.dtype)
            return f

        xcopies = [pltpu.make_async_copy(x.at[0], xbuf.at[t], xsem.at[t]) for t, x in enumerate((ax, bx))]

        def x_wait():
            for c in xcopies:
                c.wait()

        phases = [
            (16, wq_copy(0, awq), None, no_compute, None),
            (16, wq_copy(1, bwq), x_wait, q_compute(0), None),
            (128, kv_copy(ak), k_begin, k_compute(0), None),
            (128, kv_copy(av), v_begin, v_compute, None),
            (16, wo_copy(awo), wo_begin, wo_compute(functools.partial(q_part, 1)), wo_end(0)),
            (128, kv_copy(bk), k_begin, k_compute(1), None),
            (128, kv_copy(bv), v_begin, v_compute, None),
            (16, wo_copy(bwo), wo_begin, wo_compute(), wo_end(1)),
        ]
        if not compute:
            phases = [(n, c, b if b is x_wait else None, no_compute, None) for (n, c, b, _, _) in phases]
            o_ref[...] = jnp.zeros(o_ref.shape, o_ref.dtype)
        lead = [L0 if prio[j] == 0 else L1 for j in range(NS)]

        for i in range(max(L0, L1)):
            for j in range(NS):
                if i < lead[j]:
                    phases[0][1](i, j).start(priority=prio[j])
        for c in xcopies:
            c.start()

        for ph, (n, copy, begin, comp, end) in enumerate(phases):
            nxt = phases[ph + 1][1] if ph + 1 < len(phases) else None
            carry = begin() if begin is not None else None
            cuts = sorted({0, n - L0, n - L1, n})
            for lo, hi in zip(cuts[:-1], cuts[1:]):
                def body(i, carry, lo=lo):
                    gen = comp(i, carry)
                    next(gen)
                    out = None
                    for st in steps:
                        for j in st:
                            copy(i, j).wait()

                        def issue():
                            for j in st:
                                if lo + lead[j] < n:
                                    copy(i + lead[j], j).start(priority=prio[j])
                                elif nxt is not None:
                                    nxt(i + lead[j] - n, j).start(priority=prio[j])
                        if issue_first:
                            issue()
                        try:
                            next(gen)
                        except StopIteration as e:
                            out = e.value
                        if not issue_first:
                            issue()
                    return out
                carry = lax.fori_loop(lo, hi, body, carry)
            if end is not None:
                end(carry)

    def fn(*a):
        anys = pl.BlockSpec(memory_space=pl.ANY)
        return pl.pallas_call(
            kern, in_specs=[anys] * 10,
            out_specs=pl.BlockSpec(memory_space=pltpu.VMEM),
            out_shape=jax.ShapeDtypeStruct((1, 1, 2 * D), BF16),
            scratch_shapes=[
                pltpu.VMEM((2, 1, D), BF16), pltpu.VMEM((2, D, H * DH), BF16),
                pltpu.VMEM((R, NS, U, DH), BF16), pltpu.VMEM((R, 256, D), BF16),
                pltpu.VMEM((2, H, DH), F32), pltpu.VMEM((128, 8, DH), F32),
                pltpu.VMEM((4, 8, DH), F32), pltpu.VMEM((4, 8, DH), F32), pltpu.VMEM((4, 8, DH), F32),
                pltpu.SemaphoreType.DMA((R, NS)), pltpu.SemaphoreType.DMA((2,))],
            compiler_params=pltpu.CompilerParams(vmem_limit_bytes=32 * 2**20, flags=flags, **cp),
        )(*a)
    return fn


_impl = make(hs=4, prio=(0, 1, 1, 1) * 2, L0=3, L1=6, disable_bounds_checks=True)


@jax.jit
def pallas_concat_heads__mha_block_cached__gqa_block_cached__decode_kernel(
    A_x, A_k_cache, A_v_cache, A_wq, A_wo, B_x, B_k_cache, B_v_cache, B_wq, B_wo):
    return _impl(A_x, A_k_cache, A_v_cache, A_wq, A_wo, B_x, B_k_cache, B_v_cache, B_wq, B_wo)
```

```python
import functools

import jax
import jax.numpy as jnp
from jax import lax
import jax.experimental.pallas as pl
import jax.experimental.pallas.tpu as pltpu

H, SK, DH, D = 32, 4096, 128, 512

PIECES = 8
PRIORITY = (0, 1, 1, 1, 0, 1, 1, 1)
LEAD = (7, 11)
SLOTS = 16
KEYS = 64
WO_ROWS = 16
WQ_ROWS, WQ_COLS = 8, 1024
W_STEPS = 32
KV_STEPS = H * SK // (PIECES * KEYS)
VPU_STEPS = 2


def _kernel(a_x, a_k, a_v, a_wq, a_wo, b_x, b_k, b_v, b_wq, b_wo, out_ref,
            x_buf, wq_buf, a_k_buf, a_v_buf, b_k_buf, b_v_buf, wo_buf,
            q_ref, s_ref, m_ref, l_ref, o_ref, rolled_ref, col_ref, sems, x_sems):
    f32, bf16 = jnp.float32, jnp.bfloat16
    row = lax.broadcasted_iota(jnp.int32, (8, DH), 0)
    lane = lax.broadcasted_iota(jnp.int32, (8, DH), 1)

    def slot(n):
        return n & (SLOTS - 1)

    def head_group(n):
        return (n & 1) + 2 * (n >> 7)

    def wq_step(t, wq, n):
        idx = (slice(None),
               pl.ds(pl.multiple_of((n >> 2) * WQ_ROWS, WQ_ROWS), WQ_ROWS),
               pl.ds(pl.multiple_of((n & 3) * WQ_COLS, WQ_COLS), WQ_COLS))
        return wq.at[idx], wq_buf.at[(t,) + idx]

    def kv_step(cache, buf, n):
        keys = pl.ds(pl.multiple_of(((n >> 1) & 63) * KEYS, KEYS), KEYS)
        return cache.at[head_group(n), :, keys], buf.at[slot(n)]

    def wo_step(wo, n):
        rows = pl.ds(pl.multiple_of(n * WO_ROWS, WO_ROWS), WO_ROWS)
        return wo.at[:, rows], wo_buf.at[slot(n)]

    def start(step, n, j):
        src, dst = step(n)
        pltpu.make_async_copy(src.at[j], dst.at[j], sems.at[slot(n)]).start(priority=PRIORITY[j])

    def wait(step, n):
        _, dst = step(n)
        pltpu.make_async_copy(dst, dst, sems.at[slot(n)]).wait()

    x_copies = [pltpu.make_async_copy(x.at[0], x_buf.at[t], x_sems.at[t])
                for t, x in enumerate((a_x, b_x))]

    def q_begin():
        for copy in x_copies:
            copy.wait()

    def q_head(t, h, carry=None):
        x = jnp.broadcast_to(x_buf[t], (8, D))
        w = wq_buf[t, :, :, pl.ds(pl.multiple_of(h * DH, DH), DH)].reshape(D, DH)
        q_ref[t, pl.ds(h, 1), :] = jnp.dot(x, w, preferred_element_type=f32)[0:1]

    def head_pairs(buf, n):
        pieces = buf[slot(n)].reshape(PIECES * KEYS, DH)
        return [pieces[2 * KEYS * k:2 * KEYS * (k + 1)] for k in range(PIECES // 2)]

    def k_begin():
        m_ref[...] = jnp.full(m_ref.shape, -jnp.inf, f32)

    def k_step(t, buf, n, carry):
        g = head_group(n)
        q = q_ref[t, pl.ds(pl.multiple_of(g * 8, 8), 8), :].astype(bf16)
        s = jnp.full((8, DH), -jnp.inf, f32)
        for k, pair in enumerate(head_pairs(buf, n)):
            qk = lax.dot_general(q, pair, (((1,), (1,)), ((), ())), preferred_element_type=f32)
            s = jnp.where(row == 2 * k + (lane >> 6), qk, s)
        s = s * (DH ** -0.5)
        s_ref[n] = s
        m_ref[g] = jnp.maximum(m_ref[g], s)

    def v_begin():
        for g in range(4):
            m_ref[g] = jnp.broadcast_to(jnp.max(m_ref[g], axis=-1, keepdims=True), (8, DH))
        l_ref[...] = jnp.zeros(l_ref.shape, f32)
        o_ref[...] = jnp.zeros(o_ref.shape, f32)

    def v_step(buf, n, carry):
        g = head_group(n)
        p = jnp.exp(s_ref[n] - m_ref[g])
        l_ref[g] += p
        p = p.astype(bf16)
        o = None
        for k, pair in enumerate(head_pairs(buf, n)):
            pv = jnp.dot(p, pair, preferred_element_type=f32)
            o = pv if o is None else jnp.where((row >> 1) == k, pv, o)
        o_ref[g] += o

    def wo_begin():
        for g in range(4):
            o = o_ref[g]
            inv = 1.0 / jnp.sum(l_ref[g], axis=-1, keepdims=True)
            for k in range(PIECES):
                rolled_ref[k, 8 * g:8 * g + 8] = (pltpu.roll(o, WO_ROWS * k, 1) if k else o) * inv
        return jnp.zeros((8, D), f32)

    def wo_lhs(n):
        lhs = None
        for j in range(PIECES):
            piece = rolled_ref[(j - n) & 7, pl.ds(4 * j + (n >> 3), 1), :]
            piece = jnp.broadcast_to(piece, (8, DH))
            lhs = piece if lhs is None else jnp.where((lane >> 4) == j, piece, lhs)
        return lhs.astype(bf16)

    def wo_mxu(n, acc):
        w = wo_buf[slot(n)].reshape(PIECES * WO_ROWS, D)
        return acc + jnp.dot(wo_lhs(n), w, preferred_element_type=f32)

    def a_wo_step(n, acc):
        acc = wo_mxu(n, acc)
        q_head(1, n)
        return acc

    def a_end(acc):
        out_ref[0, :, 0:D] = acc[0:1].astype(out_ref.dtype)

    def b_wo_begin():
        acc = wo_begin()
        for k in range(VPU_STEPS):
            lhs = wo_lhs(W_STEPS - VPU_STEPS + k).astype(f32)
            col_ref[k] = jnp.broadcast_to(lhs[0:1], (DH, DH)).T
        return acc

    def b_end(acc):
        parts = [jnp.where(row == 0, acc[:, c:c + DH], 0.0) for c in range(0, D, DH)]
        for k in range(VPU_STEPS):
            n = W_STEPS - VPU_STEPS + k
            wait(functools.partial(wo_step, b_wo), n)
            for j in range(PIECES):
                w = wo_buf[slot(n), j].astype(f32)
                col = col_ref[k, WO_ROWS * j:WO_ROWS * (j + 1)]
                for c in range(D // DH):
                    prod = w[:, DH * c:DH * (c + 1)] * col
                    parts[c] = parts[c] + (prod[:8] + prod[8:])
        total = jnp.sum(jnp.concatenate(parts, axis=1), axis=0, keepdims=True)
        out_ref[0, :, D:2 * D] = total.astype(out_ref.dtype)

    part = functools.partial
    phases = [
        (W_STEPS, part(wq_step, 0, a_wq), None, None, None),
        (W_STEPS, part(wq_step, 1, b_wq), q_begin, part(q_head, 0), None),
        (KV_STEPS, part(kv_step, a_k, a_k_buf), k_begin, part(k_step, 0, a_k_buf), None),
        (KV_STEPS, part(kv_step, a_v, a_v_buf), v_begin, part(v_step, a_v_buf), None),
        (W_STEPS, part(wo_step, a_wo), wo_begin, a_wo_step, a_end),
        (KV_STEPS, part(kv_step, b_k, b_k_buf), k_begin, part(k_step, 1, b_k_buf), None),
        (KV_STEPS, part(kv_step, b_v, b_v_buf), v_begin, part(v_step, b_v_buf), None),
        (W_STEPS, part(wo_step, b_wo), b_wo_begin, wo_mxu, b_end),
    ]

    for n in range(max(LEAD)):
        for j in range(PIECES):
            if n < LEAD[PRIORITY[j]]:
                start(phases[0][1], n, j)
    for copy in x_copies:
        copy.start(priority=1)

    def run_step(steps, step, following, compute, first, n, carry):
        wait(step, n)
        if compute is not None:
            carry = compute(n, carry)
        for j in range(PIECES):
            lead = LEAD[PRIORITY[j]]
            if first + lead < steps:
                start(step, n + lead, j)
            elif following is not None:
                start(following, n + lead - steps, j)
        return carry

    for i, (steps, step, begin, compute, end) in enumerate(phases):
        following = phases[i + 1][1] if i + 1 < len(phases) else None
        stop = steps if following is not None else steps - VPU_STEPS
        carry = begin() if begin is not None else None
        cuts = (0, steps - LEAD[1], steps - LEAD[0], stop)
        for lo, hi in zip(cuts[:-1], cuts[1:]):
            carry = lax.fori_loop(lo, hi, part(run_step, steps, step, following, compute, lo), carry)
        if end is not None:
            end(carry)


@jax.jit
def pallas_concat_heads__mha_block_cached__gqa_block_cached__decode_kernel(
    A_x: jax.Array,
    A_k_cache: jax.Array,
    A_v_cache: jax.Array,
    A_wq: jax.Array,
    A_wo: jax.Array,
    B_x: jax.Array,
    B_k_cache: jax.Array,
    B_v_cache: jax.Array,
    B_wq: jax.Array,
    B_wo: jax.Array,
):
    def views(x, k_cache, v_cache, wq, wo):
        return (x,
                k_cache.reshape(H // PIECES, PIECES, SK, DH),
                v_cache.reshape(H // PIECES, PIECES, SK, DH),
                wq.reshape(PIECES, D // PIECES, H * DH),
                wo.reshape(PIECES, H * DH // PIECES, D))

    f32, bf16 = jnp.float32, jnp.bfloat16
    return pl.pallas_call(
        _kernel,
        in_specs=[pl.BlockSpec(memory_space=pl.ANY)] * 10,
        out_specs=pl.BlockSpec(memory_space=pltpu.VMEM),
        out_shape=jax.ShapeDtypeStruct((1, 1, 2 * D), A_x.dtype),
        scratch_shapes=[
            pltpu.VMEM((2, 1, D), bf16),
            pltpu.VMEM((2, PIECES, D // PIECES, H * DH), bf16),
            *[pltpu.VMEM((SLOTS, PIECES, KEYS, DH), bf16)] * 4,
            pltpu.VMEM((SLOTS, PIECES, WO_ROWS, D), bf16),
            pltpu.VMEM((2, H, DH), f32),
            pltpu.VMEM((KV_STEPS, 8, DH), f32),
            pltpu.VMEM((4, 8, DH), f32),
            pltpu.VMEM((4, 8, DH), f32),
            pltpu.VMEM((4, 8, DH), f32),
            pltpu.VMEM((PIECES, H, DH), f32),
            pltpu.VMEM((VPU_STEPS, DH, DH), f32),
            pltpu.SemaphoreType.DMA((SLOTS,)),
            pltpu.SemaphoreType.DMA((2,)),
        ],
        compiler_params=pltpu.CompilerParams(
            vmem_limit_bytes=32 * 1024 * 1024,
            disable_semaphore_checks=True,
        ),
    )(*views(A_x, A_k_cache, A_v_cache, A_wq, A_wo),
      *views(B_x, B_k_cache, B_v_cache, B_wq, B_wo))
```
